```python
import jax
import jax.numpy as jnp

def _softmax(x, axis=-1):
    return jax.nn.softmax(x, axis=axis)

def _gelu(x):
    return jax.nn.gelu(x, approximate=True)

def _silu(x):
    return jax.nn.silu(x)

def _sigmoid(x):
    return jax.nn.sigmoid(x)

def _layernorm(x, axis=-1, eps=1e-05):
    m = jnp.mean(x, axis=axis, keepdims=True)
    v = jnp.var(x, axis=axis, keepdims=True)
    return (x - m) / jnp.sqrt(v + eps)

def _scatter_add(tgt, idx, src, axis=0):
    return tgt.at[idx].add(src)

def _segment_sum(src, seg, n):
    return jax.ops.segment_sum(src, seg, n)

class _Rng:

    def __init__(self, key):
        self._k = key

    def _next(self):
        self._k, sub = jax.random.split(self._k)
        return sub

    def normal(self, shape):
        return jax.random.normal(self._next(), shape, dtype=jnp.bfloat16)

    def randint(self, lo, hi, shape):
        return jax.random.randint(self._next(), shape, lo, hi, dtype=jnp.int32)

    def uniform(self, shape, lo=0.0, hi=1.0):
        return jax.random.uniform(self._next(), shape, jnp.bfloat16, lo, hi)

    def permutation(self, n):
        return jax.random.permutation(self._next(), n)
kernel_name = 'adaLN_cond__sliding_block_cached__dense_activation_mish__decode'

def setup_inputs():
    _rng = _Rng(jax.random.key(int.from_bytes(__import__("os").urandom(4), "little")))
    _w = lambda a: (lambda t: t.astype(jnp.bfloat16) if jnp.issubdtype(t.dtype, jnp.floating) else t)(jnp.asarray(a))

    def _A_setup():
        B, Sq, D = (1, 1, 640)
        Hq, Hkv, Sk, Dh = (32, 32, 32768, 192)
        assert Hq % Hkv == 0, (Hq, Hkv)
        return {'x': _w((lambda *s: _rng.normal(s) * 0.05)(B, Sq, D)), 'k_cache': _w((lambda *s: _rng.normal(s) * 0.05)(B, Hkv, Sk, Dh)), 'v_cache': _w((lambda *s: _rng.normal(s) * 0.05)(B, Hkv, Sk, Dh)), 'wq': _w((lambda *s: _rng.normal(s) * 0.05)(D, Hq * Dh) * D ** (-0.5)), 'wo': _w((lambda *s: _rng.normal(s) * 0.05)(Hq * Dh, D) * (Hq * Dh) ** (-0.5))}
    _A_in = _A_setup()

    def _B_setup():
        B, S, D, F = (1, 1, 640, 1536)
        return {'x': _w((lambda *s: _rng.normal(s) * 0.05)(B, S, D)), 'w1': _w((lambda *s: _rng.normal(s) * 0.05)(D, F) * D ** (-0.5)), 'b1': _w((lambda *s: _rng.normal(s) * 0.05)(F)), 'w2': _w((lambda *s: _rng.normal(s) * 0.05)(F, D) * F ** (-0.5))}
    _B_in = _B_setup()
    return {'A_x': _A_in['x'], 'A_k_cache': _A_in['k_cache'], 'A_v_cache': _A_in['v_cache'], 'A_wq': _A_in['wq'], 'A_wo': _A_in['wo'], 'B_x': _B_in['x'], 'B_w1': _B_in['w1'], 'B_b1': _B_in['b1'], 'B_w2': _B_in['w2'], 'c': _w((lambda *s: _rng.normal(s) * 0.05)(1, 640)), 'w_mod': _w((lambda *s: _rng.normal(s) * 0.05)(640, 6 * 640) * 640 ** (-0.5))}

def reference(A_x, A_k_cache, A_v_cache, A_wq, A_wo, B_x, B_w1, B_b1, B_w2, c, w_mod):

    def _A_ref(x, k_cache, v_cache, wq, wo):
        B, Sq, D = x.shape
        Hq, Dh = (32, 192)
        Hkv, Sk = (k_cache.shape[1], k_cache.shape[2])
        W = min(4096, max(256, Sk // 4))
        rep = Hq // Hkv
        q = (lambda x, *d: x.transpose(*d))((x @ wq).reshape(B, Sq, Hq, Dh), 0, 2, 1, 3)
        k = jnp.repeat(k_cache[:, :, Sk - W:, :], rep, axis=1)
        v = jnp.repeat(v_cache[:, :, Sk - W:, :], rep, axis=1)
        scores = jnp.einsum('bhqd,bhkd->bhqk', q, k) * Dh ** (-0.5)
        p = _softmax(scores, axis=-1)
        o = jnp.einsum('bhqk,bhkd->bhqd', p, v)
        return (lambda x, *d: x.transpose(*d))(o, 0, 2, 1, 3).reshape(B, Sq, Hq * Dh) @ wo

    def _B_ref(x, w1, b1, w2):
        h = jnp.einsum('bsd,df->bsf', x, w1) + b1
        sp = jnp.log1p(jnp.exp(-jnp.abs(h))) + jnp.where(h > 0, h, jnp.zeros_like(h))
        act = h * jnp.tanh(sp)
        return jnp.einsum('bsf,fd->bsd', act, w2)
    x = A_x
    mod = (_silu(c) @ w_mod).reshape(c.shape[0], 6, 1, -1)
    sa, ca, ga, sb, cb, gb = (mod[:, 0].copy(), mod[:, 1].copy(), mod[:, 2].copy(), mod[:, 3].copy(), mod[:, 4].copy(), mod[:, 5].copy())
    h = _layernorm(x, axis=-1) * (1 + ca) + sa
    x = x + ga * _A_ref(h, A_k_cache, A_v_cache, A_wq, A_wo)
    h = _layernorm(x, axis=-1) * (1 + cb) + sb
    x = x + gb * _B_ref(h, B_w1, B_b1, B_w2)
    return x
```

```python
import jax
import jax.numpy as jnp
from jax import lax
import jax.experimental.pallas as pl
import jax.experimental.pallas.tpu as pltpu

F32 = jnp.float32
BF16 = jnp.bfloat16
M = 8
N_HEADS, HEAD_DIM = 32, 192


def _layernorm(x, eps=1e-5):
    m = jnp.mean(x, axis=-1, keepdims=True)
    d = x - m
    v = jnp.mean(d * d, axis=-1, keepdims=True)
    return d / jnp.sqrt(v + eps)


def _dot(a, b):
    return jnp.dot(a, b, preferred_element_type=F32)


def _dot_nt(a, b):
    return lax.dot_general(a, b, (((1,), (1,)), ((), ())), preferred_element_type=F32)


@jax.jit
def pallas_adaLN_cond__sliding_block_cached__dense_activation_mish__decode_kernel(
    A_x: jax.Array,
    A_k_cache: jax.Array,
    A_v_cache: jax.Array,
    A_wq: jax.Array,
    A_wo: jax.Array,
    B_x: jax.Array,
    B_w1: jax.Array,
    B_b1: jax.Array,
    B_w2: jax.Array,
    c: jax.Array,
    w_mod: jax.Array,
):
    del B_x
    D = A_x.shape[-1]
    FF = B_w1.shape[-1]
    H, DH = N_HEADS, HEAD_DIM
    SK = A_k_cache.shape[2]
    W = min(4096, max(256, SK // 4))
    G = 2
    R = G * DH
    NP = H // G
    NBUF = 4

    def kernel(x_hbm, kt_hbm, vt_hbm, wq_hbm, wo_hbm, w1_hbm, b1_hbm, w2_hbm, c_hbm, wmod_hbm,
               o_ref,
               x_v, c_v, b1_v, wmod_v, wq_v, wo_v, w1_v, w2_v, kbuf, vbuf, q_v, acc_v,
               wsem, ksem, vsem):
        def kv_copy(src, buf, sem, p, slot):
            return pltpu.make_async_copy(
                src.at[pl.ds(pl.multiple_of(p * R, R), R), pl.ds(SK - W, W)],
                buf.at[slot], sem.at[slot])

        cp_c = pltpu.make_async_copy(c_hbm, c_v, wsem.at[0])
        cp_x = pltpu.make_async_copy(x_hbm.at[0], x_v, wsem.at[1])
        cp_b1 = pltpu.make_async_copy(b1_hbm, b1_v, wsem.at[2])
        cp_wmod = pltpu.make_async_copy(wmod_hbm, wmod_v, wsem.at[3])
        cp_wq = pltpu.make_async_copy(wq_hbm, wq_v, wsem.at[4])
        cp_wo = pltpu.make_async_copy(wo_hbm, wo_v, wsem.at[5])
        cp_w1 = pltpu.make_async_copy(w1_hbm, w1_v, wsem.at[6])
        cp_w2 = pltpu.make_async_copy(w2_hbm, w2_v, wsem.at[7])

        cp_wmod.start()
        cp_c.start()
        cp_x.start()
        cp_b1.start()
        cp_wq.start()
        for j in range(NBUF):
            kv_copy(kt_hbm, kbuf, ksem, j, j).start()
            kv_copy(vt_hbm, vbuf, vsem, j, j).start()
            if j == 0:
                cp_wo.start()

        cp_c.wait()
        cp_x.wait()
        cp_b1.wait()
        cp_wmod.wait()
        cc = jnp.broadcast_to(c_v[...].astype(F32), (M, D))
        sc = (cc * jax.nn.sigmoid(cc)).astype(BF16)
        mod = _dot(sc, wmod_v[...])
        sa, ca, ga, sb, cb, gb = (mod[:, i * D:(i + 1) * D] for i in range(6))
        x = jnp.broadcast_to(x_v[...].astype(F32), (M, D))
        h = (_layernorm(x) * (1.0 + ca) + sa).astype(BF16)
        cp_wq.wait()
        q = _dot(h, wq_v[...])
        row = lax.broadcasted_iota(jnp.int32, (M, R), 0)
        col = lax.broadcasted_iota(jnp.int32, (M, R), 1)
        diag = (col >= row * DH) & (col < (row + 1) * DH)
        for p in range(NP):
            q_v[p] = jnp.where(diag, q[:, p * R:(p + 1) * R], 0.0).astype(BF16)
        acc_v[...] = jnp.zeros_like(acc_v)
        cp_wo.wait()

        def body(p, carry):
            slot = p % NBUF
            kv_copy(kt_hbm, kbuf, ksem, p, slot).wait()
            s = _dot(q_v[p], kbuf[slot]) * (DH ** -0.5)

            @pl.when(p + NBUF < NP)
            def _():
                kv_copy(kt_hbm, kbuf, ksem, p + NBUF, slot).start()

            m = jnp.max(s, axis=-1, keepdims=True)
            e = jnp.exp(s - m)
            l = jnp.sum(e, axis=-1, keepdims=True)
            pr = (e / l).astype(BF16)
            kv_copy(vt_hbm, vbuf, vsem, p, slot).wait()
            o = _dot_nt(pr, vbuf[slot])

            @pl.when(p + NBUF < NP)
            def _():
                kv_copy(vt_hbm, vbuf, vsem, p + NBUF, slot).start()

            @pl.when(p + NBUF == NP)
            def _():
                cp_w1.start()
                cp_w2.start()

            o = jnp.where(diag, o, 0.0).astype(BF16)
            acc_v[...] += _dot(o, wo_v[pl.ds(pl.multiple_of(p * R, R), R), :])
            return carry

        lax.fori_loop(0, NP, body, 0)

        a = jnp.sum(acc_v[...], axis=0, keepdims=True)
        x1 = x + ga * a
        h2 = (_layernorm(x1) * (1.0 + cb) + sb).astype(BF16)
        cp_w1.wait()
        b1 = b1_v[...].astype(F32).reshape(1, FF)
        u = _dot(h2, w1_v[...]) + b1
        sp = jnp.log1p(jnp.exp(-jnp.abs(u))) + jnp.where(u > 0, u, 0.0)
        act = (u * jnp.tanh(sp)).astype(BF16)
        cp_w2.wait()
        y = _dot(act, w2_v[...])
        out = x1 + gb * y
        o_ref[0] = out[0:1, :].astype(o_ref.dtype)

    kt = jnp.swapaxes(A_k_cache, 2, 3).reshape(H * DH, SK)
    vt = jnp.swapaxes(A_v_cache, 2, 3).reshape(H * DH, SK)
    return pl.pallas_call(
        kernel,
        out_shape=jax.ShapeDtypeStruct(A_x.shape, A_x.dtype),
        in_specs=[pl.BlockSpec(memory_space=pltpu.HBM)] * 10,
        out_specs=pl.BlockSpec(memory_space=pltpu.VMEM),
        scratch_shapes=[
            pltpu.VMEM((1, D), BF16), pltpu.VMEM((1, D), BF16), pltpu.VMEM((FF,), BF16),
            pltpu.VMEM((D, 6 * D), BF16), pltpu.VMEM((D, H * DH), BF16),
            pltpu.VMEM((H * DH, D), BF16), pltpu.VMEM((D, FF), BF16), pltpu.VMEM((FF, D), BF16),
            pltpu.VMEM((NBUF, R, W), BF16), pltpu.VMEM((NBUF, R, W), BF16),
            pltpu.VMEM((NP, M, R), BF16), pltpu.VMEM((M, D), F32),
            pltpu.SemaphoreType.DMA((8,)), pltpu.SemaphoreType.DMA((NBUF,)),
            pltpu.SemaphoreType.DMA((NBUF,)),
        ],
        compiler_params=pltpu.CompilerParams(vmem_limit_bytes=100 * 1024 * 1024),
    )(A_x, kt, vt, A_wq, A_wo, B_w1, B_b1, B_w2, c, w_mod)
```

```python
import functools
import jax
import jax.numpy as jnp
from jax import lax
from jax.experimental import pallas as pl
from jax.experimental.pallas import tpu as pltpu

F32 = jnp.float32
BF16 = jnp.bfloat16
M = 8


def _layernorm(x, eps=1e-5):
    m = jnp.mean(x, axis=-1, keepdims=True)
    d = x - m
    v = jnp.mean(d * d, axis=-1, keepdims=True)
    return d / jnp.sqrt(v + eps)


def _dot(a, b):
    return jnp.dot(a, b, preferred_element_type=F32)


def _dot_nt(a, b):
    return lax.dot_general(a, b, (((1,), (1,)), ((), ())), preferred_element_type=F32)


def make(unroll=2, nobounds=True, w2_groups=4, dma_only=False):
    D, H, DH, SK, FF = 640, 32, 192, 32768, 1536
    W = min(4096, max(256, SK // 4))
    G = 2
    R = G * DH
    NP = H // G
    NB = 2

    def kernel(x_hbm, kt_hbm, vt_hbm, wq_hbm, wo_hbm, w1_hbm, b1_hbm, w2_hbm, c_hbm, wmod_hbm,
               o_ref,
               x_v, c_v, b1_v, wmod_v, wq_v, wo_v, w1_v, w2_v, kbuf, vbuf, p_v, acc_v,
               wsem, w2sem, ksem, vsem, osem):

        def start(src, dst, sem, r, nr, c0, nc, prio, dr=None, dc=None):
            dr = r if dr is None else dr
            dc = c0 if dc is None else dc
            pltpu.make_async_copy(
                src.at[pl.ds(pl.multiple_of(r, 8), nr), pl.ds(c0, nc)],
                dst.at[pl.ds(pl.multiple_of(dr, 8), nr), pl.ds(dc, nc)], sem).start(priority=prio)

        def wait_all(buf, sem):
            pltpu.make_async_copy(buf, buf, sem).wait()

        def loop(lo, hi, f):
            lax.fori_loop(0, hi - lo, lambda i, c: (f(i + lo), c)[1], 0, unroll=unroll)

        def issue_wmod():
            def f(i):
                start(wmod_hbm, wmod_v, wsem.at[3], i * 8, 8, 0, 1920, 0)
                start(wmod_hbm, wmod_v, wsem.at[3], i * 8, 8, 1920, 1920, 1)
            loop(0, D // 8, f)

        def issue_wq():
            def f(i):
                for j in range(3):
                    start(wq_hbm, wq_v, wsem.at[4], i * 8, 8, j * 2048, 2048, 0)
                    start(wq_hbm, wq_v, wsem.at[4], i * 8 + D // 2, 8, j * 2048, 2048, 1)
            loop(0, D // 16, f)

        def issue_kv(p, half):
            slot = p % NB

            def f(i):
                for j in range(2):
                    start(kt_hbm, kbuf.at[slot], ksem.at[slot], p * R + i * 8, 8, SK - W + j * 2048, 2048, 0,
                          dr=i * 8, dc=j * 2048)
                    start(vt_hbm, vbuf.at[slot], vsem.at[slot], p * R + i * 8, 8, SK - W + j * 2048, 2048, 1,
                          dr=i * 8, dc=j * 2048)
            n = R // 16
            loop(half * n, (half + 1) * n, f)

            def g(i):
                start(wo_hbm, wo_v.at[slot], osem.at[slot], p * R + i * 24, 24, 0, D, 0, dr=i * 24)
                start(wo_hbm, wo_v.at[slot], osem.at[slot], p * R + i * 24 + R // 2, 24, 0, D, 1, dr=i * 24 + R // 2)
            loop(half * 4, (half + 1) * 4, g)

        def issue_w1():
            def f(i):
                start(w1_hbm, w1_v, wsem.at[5], i * 8, 8, 0, FF, 0)
                start(w1_hbm, w1_v, wsem.at[5], i * 8 + D // 2, 8, 0, FF, 1)
            loop(0, D // 16, f)

        RG = FF // w2_groups

        def issue_w2():
            def f(i):
                g = i // (RG // 48)
                start(w2_hbm, w2_v, w2sem.at[g], i * 48, 24, 0, D, 0)
                start(w2_hbm, w2_v, w2sem.at[g], i * 48 + 24, 24, 0, D, 1)
            loop(0, FF // 48, f)

        cp_c = pltpu.make_async_copy(c_hbm, c_v, wsem.at[0])
        cp_x = pltpu.make_async_copy(x_hbm.at[0], x_v, wsem.at[1])
        cp_b1 = pltpu.make_async_copy(b1_hbm, b1_v, wsem.at[2])
        cp_c.start()
        cp_x.start()
        cp_b1.start()
        issue_wmod()
        issue_wq()

        cp_c.wait()
        cp_x.wait()
        cp_b1.wait()
        wait_all(wmod_v, wsem.at[3])
        if not dma_only:
            c = jnp.broadcast_to(c_v[...].astype(F32), (M, D))
            sc = (c * jax.nn.sigmoid(c)).astype(BF16)
            mod = _dot(sc, wmod_v[...])
            sa, ca, ga, sb, cb, gb = (mod[:, i * D:(i + 1) * D] for i in range(6))
            x = jnp.broadcast_to(x_v[...].astype(F32), (M, D))
            h = (_layernorm(x) * (1.0 + ca) + sa).astype(BF16)
        row = lax.broadcasted_iota(jnp.int32, (M, R), 0)
        col = lax.broadcasted_iota(jnp.int32, (M, R), 1)
        diag = (col >= row * DH) & (col < (row + 1) * DH)
        acc_v[...] = jnp.zeros_like(acc_v)

        issue_kv(0, 0)
        issue_kv(0, 1)
        wait_all(wq_v, wsem.at[4])

        def body(p, carry):
            slot = p % NB

            @pl.when(p + 1 < NP)
            def _():
                issue_kv(p + 1, 0)

            @pl.when(p + 1 == NP)
            def _():
                issue_w1()

            wait_all(kbuf.at[slot], ksem.at[slot])
            if not dma_only:
                q = _dot(h, wq_v[:, pl.ds(pl.multiple_of(p * R, 128), R)])
                q = jnp.where(diag, q, 0.0).astype(BF16)
                s = _dot(q, kbuf[slot]) * (DH ** -0.5)
                m = jnp.max(s, axis=-1, keepdims=True)
                e = jnp.exp(s - m)
                l = jnp.sum(e, axis=-1, keepdims=True)
                p_v[...] = e / l

            @pl.when(p + 1 < NP)
            def _():
                issue_kv(p + 1, 1)

            @pl.when(p + 1 == NP)
            def _():
                issue_w2()

            wait_all(vbuf.at[slot], vsem.at[slot])
            wait_all(wo_v.at[slot], osem.at[slot])
            if not dma_only:
                o = _dot_nt(p_v[...].astype(BF16), vbuf[slot])
                o = jnp.where(diag, o, 0.0).astype(BF16)
                acc_v[...] += _dot(o, wo_v[slot])
            return carry

        lax.fori_loop(0, NP, body, 0)

        wait_all(w1_v, wsem.at[5])
        if not dma_only:
            a = jnp.sum(acc_v[...], axis=0, keepdims=True)
            x1 = x + ga * a
            h2 = (_layernorm(x1) * (1.0 + cb) + sb).astype(BF16)
            b1 = b1_v[...].astype(F32).reshape(1, FF)
            u = _dot(h2, w1_v[...]) + b1
            sp = jnp.log1p(jnp.exp(-jnp.abs(u))) + jnp.where(u > 0, u, 0.0)
            act = (u * jnp.tanh(sp)).astype(BF16)
        y = jnp.zeros((M, D), F32)
        for g in range(w2_groups):
            wait_all(w2_v.at[pl.ds(g * RG, RG)], w2sem.at[g])
            if not dma_only:
                y += _dot(act[:, g * RG:(g + 1) * RG], w2_v[g * RG:(g + 1) * RG, :])
        if not dma_only:
            out = x1 + gb * y
        else:
            out = y
        o_ref[0] = out[0:1, :].astype(o_ref.dtype)

    def fn(A_x, A_k_cache, A_v_cache, A_wq, A_wo, B_x, B_w1, B_b1, B_w2, c, w_mod):
        kt = jnp.swapaxes(A_k_cache, 2, 3).reshape(H * DH, SK)
        vt = jnp.swapaxes(A_v_cache, 2, 3).reshape(H * DH, SK)
        return pl.pallas_call(
            kernel,
            out_shape=jax.ShapeDtypeStruct((1, 1, D), BF16),
            in_specs=[pl.BlockSpec(memory_space=pltpu.HBM)] * 10,
            out_specs=pl.BlockSpec(memory_space=pltpu.VMEM),
            scratch_shapes=[
                pltpu.VMEM((1, D), BF16), pltpu.VMEM((1, D), BF16), pltpu.VMEM((FF,), BF16),
                pltpu.VMEM((D, 6 * D), BF16), pltpu.VMEM((D, H * DH), BF16),
                pltpu.VMEM((NB, R, D), BF16), pltpu.VMEM((D, FF), BF16), pltpu.VMEM((FF, D), BF16),
                pltpu.VMEM((NB, R, W), BF16), pltpu.VMEM((NB, R, W), BF16),
                pltpu.VMEM((M, W), F32), pltpu.VMEM((M, D), F32),
                pltpu.SemaphoreType.DMA((6,)), pltpu.SemaphoreType.DMA((w2_groups,)),
                pltpu.SemaphoreType.DMA((NB,)), pltpu.SemaphoreType.DMA((NB,)), pltpu.SemaphoreType.DMA((NB,)),
            ],
            compiler_params=pltpu.CompilerParams(vmem_limit_bytes=100 * 1024 * 1024,
                                                 disable_bounds_checks=nobounds),
        )(A_x, kt, vt, A_wq, A_wo, B_w1, B_b1, B_w2, c, w_mod)
    return fn


@jax.jit
def pallas_adaLN_cond__sliding_block_cached__dense_activation_mish__decode_kernel(A_x, A_k_cache, A_v_cache, A_wq, A_wo, B_x, B_w1, B_b1, B_w2, c, w_mod):
    return make(unroll=True, nobounds=False)(A_x, A_k_cache, A_v_cache, A_wq, A_wo, B_x, B_w1, B_b1, B_w2, c, w_mod)
```

```python
import functools
import jax
import jax.numpy as jnp
from jax import lax
from jax.experimental import pallas as pl
from jax.experimental.pallas import tpu as pltpu

F32 = jnp.float32
BF16 = jnp.bfloat16
M = 8


def _layernorm(x, eps=1e-5):
    m = jnp.mean(x, axis=-1, keepdims=True)
    d = x - m
    v = jnp.mean(d * d, axis=-1, keepdims=True)
    return d / jnp.sqrt(v + eps)


def _dot(a, b):
    return jnp.dot(a, b, preferred_element_type=F32)


def _dot_nt(a, b):
    return lax.dot_general(a, b, (((1,), (1,)), ((), ())), preferred_element_type=F32)


def seq(name, rows, nr, cols, r0=0):
    out = []
    for r in range(r0, rows, nr):
        c = 0
        for nc in cols:
            out.append((name, r, nr, c, nc))
            c += nc
    return out


def strided(lst, k):
    return [lst[i] for s in range(k) for i in range(s, len(lst), k)]


def altp(lst):
    return [(*x, i % 2) for i, x in enumerate(lst)]


def merge(*lists):
    tagged = []
    for j, l in enumerate(lists):
        for i, x in enumerate(l):
            tagged.append(((i + 0.5) / len(l), j, x))
    tagged.sort(key=lambda t: (t[0], t[1]))
    return [t[2] for t in tagged]


def pairs(lst):
    return [lst[i:i + 2] for i in range(0, len(lst), 2)]


def make(nobounds=True, w2_groups=4, dma_only=False, kv_rows=32, kv_cols=512, s_wmod=26, s_wq=24,
         s_w1=20, s_w2=4, wo_rows=24, wo_mode="merge", small_at=2):
    D, H, DH, SK, FF = 640, 32, 192, 32768, 1536
    W = min(4096, max(256, SK // 4))
    G = 2
    R = G * DH
    NP = H // G
    NB = 2
    RG = FF // w2_groups

    pro = altp(strided(seq("wmod", D, 8, [1920, 1920]), s_wmod)) + altp(strided(seq("wq", D, 8, [2048] * 3), s_wq))
    kv = []
    for c in range(0, W, kv_cols):
        for r in range(0, R, kv_rows):
            kv.append([("k", r, kv_rows, c, kv_cols, 0), ("v", r, kv_rows, c, kv_cols, 1)])
    wo = pairs(altp(seq("wo", R, wo_rows, [D])))
    if wo_mode == "merge":
        step = sum(merge(kv, wo), [])
    elif wo_mode == "end":
        step = sum(kv + wo, [])
    half = len(step) // 4 * 2
    step_a, step_b = step[:half], step[half:]
    tail_a = altp(strided(seq("w1", D, 8, [FF]), s_w1))
    tail_b = sum([altp(strided(seq(("w2", g), (g + 1) * RG, 24, [D], r0=g * RG), s_w2)) for g in range(w2_groups)], [])

    def kernel(x_hbm, kt_hbm, vt_hbm, wq_hbm, wo_hbm, w1_hbm, b1_hbm, w2_hbm, c_hbm, wmod_hbm,
               o_ref,
               x_v, c_v, b1_v, wmod_v, wq_v, wo_v, w1_v, w2_v, kbuf, vbuf, p_v, acc_v,
               wsem, w2sem, ksem, vsem, osem):

        def issue(pieces, p=None):
            if p is not None:
                slot = p % NB
                base = p * R if isinstance(p, int) else pl.multiple_of(p * R, R)
            for (name, r, nr, c, nc, prio) in pieces:
                if name == "k":
                    src, dst, sem = kt_hbm.at[pl.ds(base + r, nr), pl.ds(SK - W + c, nc)], kbuf.at[slot], ksem.at[slot]
                elif name == "v":
                    src, dst, sem = vt_hbm.at[pl.ds(base + r, nr), pl.ds(SK - W + c, nc)], vbuf.at[slot], vsem.at[slot]
                elif name == "wo":
                    src, dst, sem = wo_hbm.at[pl.ds(base + r, nr), pl.ds(c, nc)], wo_v.at[slot], osem.at[slot]
                else:
                    if name == "wmod":
                        s, dst, sem = wmod_hbm, wmod_v, wsem.at[3]
                    elif name == "wq":
                        s, dst, sem = wq_hbm, wq_v, wsem.at[4]
                    elif name == "w1":
                        s, dst, sem = w1_hbm, w1_v, wsem.at[5]
                    else:
                        s, dst, sem = w2_hbm, w2_v, w2sem.at[name[1]]
                    src = s.at[pl.ds(r, nr), pl.ds(c, nc)]
                pltpu.make_async_copy(src, dst.at[pl.ds(r, nr), pl.ds(c, nc)], sem).start(priority=prio)

        def wait_all(buf, sem):
            pltpu.make_async_copy(buf, buf, sem).wait()

        cp_c = pltpu.make_async_copy(c_hbm, c_v, wsem.at[0])
        cp_x = pltpu.make_async_copy(x_hbm.at[0], x_v, wsem.at[1])
        cp_b1 = pltpu.make_async_copy(b1_hbm, b1_v, wsem.at[2])
        issue(pro[:small_at])
        cp_c.start()
        cp_x.start()
        cp_b1.start()
        issue(pro[small_at:])

        cp_c.wait()
        cp_x.wait()
        cp_b1.wait()
        wait_all(wmod_v, wsem.at[3])
        if not dma_only:
            c = jnp.broadcast_to(c_v[...].astype(F32), (M, D))
            sc = (c * jax.nn.sigmoid(c)).astype(BF16)
            mod = _dot(sc, wmod_v[...])
            sa, ca, ga, sb, cb, gb = (mod[:, i * D:(i + 1) * D] for i in range(6))
            x = jnp.broadcast_to(x_v[...].astype(F32), (M, D))
            h = (_layernorm(x) * (1.0 + ca) + sa).astype(BF16)
        row = lax.broadcasted_iota(jnp.int32, (M, R), 0)
        col = lax.broadcasted_iota(jnp.int32, (M, R), 1)
        diag = (col >= row * DH) & (col < (row + 1) * DH)
        acc_v[...] = jnp.zeros_like(acc_v)

        def body(i, carry):
            p = i - 1
            slot = p % NB

            @pl.when(i < NP)
            def _():
                issue(step_a, i)

            @pl.when(i == NP)
            def _():
                issue(tail_a)

            @pl.when(i == 0)
            def _():
                wait_all(wq_v, wsem.at[4])

            @pl.when(i > 0)
            def _():
                wait_all(kbuf.at[slot], ksem.at[slot])
                if not dma_only:
                    q = _dot(h, wq_v[:, pl.ds(pl.multiple_of(p * R, 128), R)])
                    q = jnp.where(diag, q, 0.0).astype(BF16)
                    s = _dot(q, kbuf[slot]) * (DH ** -0.5)
                    m = jnp.max(s, axis=-1, keepdims=True)
                    e = jnp.exp(s - m)
                    l = jnp.sum(e, axis=-1, keepdims=True)
                    p_v[...] = e / l

            @pl.when(i < NP)
            def _():
                issue(step_b, i)

            @pl.when(i == NP)
            def _():
                issue(tail_b)

            @pl.when(i > 0)
            def _():
                wait_all(vbuf.at[slot], vsem.at[slot])
                wait_all(wo_v.at[slot], osem.at[slot])
                if not dma_only:
                    o = _dot_nt(p_v[...].astype(BF16), vbuf[slot])
                    o = jnp.where(diag, o, 0.0).astype(BF16)
                    acc_v[...] += _dot(o, wo_v[slot])
            return carry

        lax.fori_loop(0, NP + 1, body, 0)

        wait_all(w1_v, wsem.at[5])
        if not dma_only:
            a = jnp.sum(acc_v[...], axis=0, keepdims=True)
            x1 = x + ga * a
            h2 = (_layernorm(x1) * (1.0 + cb) + sb).astype(BF16)
            b1 = b1_v[...].astype(F32).reshape(1, FF)
            u = _dot(h2, w1_v[...]) + b1
            sp = jnp.log1p(jnp.exp(-jnp.abs(u))) + jnp.where(u > 0, u, 0.0)
            act = (u * jnp.tanh(sp)).astype(BF16)
        y = jnp.zeros((M, D), F32)
        for g in range(w2_groups):
            wait_all(w2_v.at[pl.ds(g * RG, RG)], w2sem.at[g])
            if not dma_only:
                y += _dot(act[:, g * RG:(g + 1) * RG], w2_v[g * RG:(g + 1) * RG, :])
        if not dma_only:
            out = x1 + gb * y
        else:
            out = y
        o_ref[0] = out[0:1, :].astype(o_ref.dtype)

    def fn(A_x, A_k_cache, A_v_cache, A_wq, A_wo, B_x, B_w1, B_b1, B_w2, c, w_mod):
        kt = jnp.swapaxes(A_k_cache, 2, 3).reshape(H * DH, SK)
        vt = jnp.swapaxes(A_v_cache, 2, 3).reshape(H * DH, SK)
        return pl.pallas_call(
            kernel,
            out_shape=jax.ShapeDtypeStruct((1, 1, D), BF16),
            in_specs=[pl.BlockSpec(memory_space=pltpu.HBM)] * 10,
            out_specs=pl.BlockSpec(memory_space=pltpu.VMEM),
            scratch_shapes=[
                pltpu.VMEM((1, D), BF16), pltpu.VMEM((1, D), BF16), pltpu.VMEM((FF,), BF16),
                pltpu.VMEM((D, 6 * D), BF16), pltpu.VMEM((D, H * DH), BF16),
                pltpu.VMEM((NB, R, D), BF16), pltpu.VMEM((D, FF), BF16), pltpu.VMEM((FF, D), BF16),
                pltpu.VMEM((NB, R, W), BF16), pltpu.VMEM((NB, R, W), BF16),
                pltpu.VMEM((M, W), F32), pltpu.VMEM((M, D), F32),
                pltpu.SemaphoreType.DMA((6,)), pltpu.SemaphoreType.DMA((w2_groups,)),
                pltpu.SemaphoreType.DMA((NB,)), pltpu.SemaphoreType.DMA((NB,)), pltpu.SemaphoreType.DMA((NB,)),
            ],
            compiler_params=pltpu.CompilerParams(vmem_limit_bytes=100 * 1024 * 1024,
                                                 disable_bounds_checks=nobounds),
        )(A_x, kt, vt, A_wq, A_wo, B_w1, B_b1, B_w2, c, w_mod)
    return fn


@jax.jit
def pallas_adaLN_cond__sliding_block_cached__dense_activation_mish__decode_kernel(A_x, A_k_cache, A_v_cache, A_wq, A_wo, B_x, B_w1, B_b1, B_w2, c, w_mod):
    return make(wo_rows=32, nobounds=False)(A_x, A_k_cache, A_v_cache, A_wq, A_wo, B_x, B_w1, B_b1, B_w2, c, w_mod)
```

```python
import jax
import jax.numpy as jnp
from jax import lax
from jax.experimental import pallas as pl
from jax.experimental.pallas import tpu as pltpu

F32 = jnp.float32
BF16 = jnp.bfloat16
M = 8
TR = 8


def _layernorm(x, eps=1e-5):
    m = jnp.mean(x, axis=-1, keepdims=True)
    d = x - m
    v = jnp.mean(d * d, axis=-1, keepdims=True)
    return d / jnp.sqrt(v + eps)


def _dot(a, b):
    return jnp.dot(a, b, preferred_element_type=F32)


def _dot_nt(a, b):
    return lax.dot_general(a, b, (((1,), (1,)), ((), ())), preferred_element_type=F32)


def make(strict=True, nosem=False, ng2=6, wo_rows=24, wmod_cols=1280, wmod_ways=8, last=0):
    D, H, DH, SK, FF = 640, 32, 192, 32768, 1536
    W = min(4096, max(256, SK // 4))
    R = 2 * DH
    NP = H // 2
    KR, KC = 32, 512
    NG = ng2
    GR = FF // (2 * NG)
    S_KV, S_WO, S_W2 = (0, 2, 4) if strict else (0, 0, 2)

    def kernel(x_hbm, kt_hbm, vt_hbm, wq_hbm, wo_hbm, w1_hbm, b1_hbm, w2_hbm, c_hbm, wmod_hbm,
               o_ref,
               x_v, c_v, b1_v, wmod_v, wq_v, wo_v, w1_v, w2_v, kv_v, p_v, acc_v, act_v, sem):

        def start(src, dst, s, queue):
            pltpu.make_async_copy(src, dst, s).start(priority=queue)

        def wait_filled(buf, s):
            pltpu.make_async_copy(buf, buf, s).wait()

        def fetch_weight(src, dst, s, cols, ways):
            n = src.shape[0] // ways
            for r in range(0, n, TR):
                for c in range(0, src.shape[1], cols):
                    for b in range(ways):
                        idx = (pl.ds(r + b * n, TR), pl.ds(c, cols))
                        start(src.at[idx], dst.at[idx], s, b % 2)

        def fetch_pair(p, half):
            slot = p % 2
            rows = lambda r, n: pl.ds(pl.multiple_of(p * R + r, TR), n)
            blocks = W // KC
            nwo = R // wo_rows // blocks
            for j in range(half * blocks // 2, (half + 1) * blocks // 2):
                for t in range(R // KR):
                    src = (rows(t * KR, KR), pl.ds(SK - W + j * KC, KC))
                    dst = (pl.ds(t * KR, KR), pl.ds(j * KC, KC))
                    start(kt_hbm.at[src], kv_v.at[slot, 0].at[dst], sem.at[S_KV + slot], 0)
                    start(vt_hbm.at[src], kv_v.at[slot, 1].at[dst], sem.at[S_KV + slot], 1)
                    for q in range(nwo):
                        if t + 1 == (q + 1) * (R // KR) // nwo:
                            r = (j * nwo + q) * wo_rows
                            start(wo_hbm.at[rows(r, wo_rows)], wo_v.at[slot, pl.ds(r, wo_rows)],
                                  sem.at[S_WO + slot], (j * nwo + q) % 2)

        def fetch_w2(g):
            for r in range(0, GR, 32):
                for q in range(2):
                    start(w2_hbm.at[pl.ds(q * FF // 2 + g * GR + r, 32)],
                          w2_v.at[g, pl.ds(q * GR + r, 32)], sem.at[S_W2 + g], q)

        s_small, s_wmod, s_wq = (sem.at[S_W2 + 1], sem.at[S_W2], sem.at[S_W2 + 2])
        small = [pltpu.make_async_copy(c_hbm, c_v, s_small),
                 pltpu.make_async_copy(x_hbm.at[0], x_v, s_small),
                 pltpu.make_async_copy(b1_hbm, b1_v, s_small)]
        for i, cp in enumerate(small):
            cp.start(priority=(i + 1) % 2)
        fetch_weight(wmod_hbm, wmod_v, s_wmod, wmod_cols, wmod_ways)
        fetch_weight(wq_hbm, wq_v, s_wq, 2048, 10)

        for cp in small:
            cp.wait()
        wait_filled(wmod_v, s_wmod)
        c = jnp.broadcast_to(c_v[...].astype(F32), (M, D))
        mod = _dot((c * jax.nn.sigmoid(c)).astype(BF16), wmod_v[...])
        sa, ca, ga, sb, cb, gb = (mod[:, i * D:(i + 1) * D] for i in range(6))
        x = jnp.broadcast_to(x_v[...].astype(F32), (M, D))
        h = (_layernorm(x) * (1.0 + ca) + sa).astype(BF16)
        row = lax.broadcasted_iota(jnp.int32, (M, R), 0)
        col = lax.broadcasted_iota(jnp.int32, (M, R), 1)
        diag = (col >= row * DH) & (col < (row + 1) * DH)
        acc_v[...] = jnp.zeros_like(acc_v)

        def step(i, carry):
            p = jnp.maximum(i - 1, 0)
            slot = p % 2

            @pl.when(i < NP)
            def _():
                fetch_pair(i, 0)

            @pl.when(i == NP)
            def _():
                fetch_weight(w1_hbm, w1_v, sem.at[S_KV + NP % 2], FF, 4)

            @pl.when(i == 0)
            def _():
                wait_filled(wq_v, s_wq)

            @pl.when(i > 0)
            def _():
                wait_filled(kv_v.at[slot], sem.at[S_KV + slot])
                wait_filled(wo_v.at[slot], sem.at[S_WO + slot])
                q = _dot(h, wq_v[:, pl.ds(pl.multiple_of(p * R, 128), R)])
                q = jnp.where(diag, q, 0.0).astype(BF16)
                s = _dot(q, kv_v[slot, 0]) * (DH ** -0.5)
                e = jnp.exp(s - jnp.max(s, axis=-1, keepdims=True))
                p_v[...] = e / jnp.sum(e, axis=-1, keepdims=True)

            @pl.when(i < NP)
            def _():
                fetch_pair(i, 1)

            @pl.when(i == NP)
            def _():
                for g in range(NG // 2):
                    fetch_w2(g)

            @pl.when(i > 0)
            def _():
                o = _dot_nt(p_v[...].astype(BF16), kv_v[slot, 1])
                o = jnp.where(diag, o, 0.0).astype(BF16)
                acc_v[...] += _dot(o, wo_v[slot])
            return carry

        lax.fori_loop(0, NP + 1, step, 0)

        for g in range(NG // 2, NG):
            fetch_w2(g)
        x1 = x + ga * jnp.sum(acc_v[...], axis=0, keepdims=True)
        h2 = (_layernorm(x1) * (1.0 + cb) + sb).astype(BF16)
        wait_filled(w1_v, sem.at[S_KV + NP % 2])
        u = _dot(h2, w1_v[...]) + b1_v[...].astype(F32).reshape(1, FF)
        softplus = jnp.log1p(jnp.exp(-jnp.abs(u))) + jnp.where(u > 0, u, 0.0)
        act = u * jnp.tanh(softplus)
        for g in range(NG):
            for q in range(2):
                lo = q * FF // 2 + g * GR
                act_v[g, :, q * GR:(q + 1) * GR] = act[:, lo:lo + GR]

        def ffn_out(g, y):
            wait_filled(w2_v.at[g], sem.at[S_W2 + g])
            return y + _dot(act_v[g].astype(BF16), w2_v[g])

        y = lax.fori_loop(0, NG, ffn_out, jnp.zeros((M, D), F32))
        o_ref[0] = (x1 + gb * y)[0:1, :].astype(o_ref.dtype)

    def fn(A_x, A_k_cache, A_v_cache, A_wq, A_wo, B_x, B_w1, B_b1, B_w2, c, w_mod):
        kt = jnp.swapaxes(A_k_cache, 2, 3).reshape(H * DH, SK)
        vt = jnp.swapaxes(A_v_cache, 2, 3).reshape(H * DH, SK)
        return pl.pallas_call(
            kernel,
            out_shape=jax.ShapeDtypeStruct((1, 1, D), BF16),
            in_specs=[pl.BlockSpec(memory_space=pltpu.HBM)] * 10,
            out_specs=pl.BlockSpec(memory_space=pltpu.VMEM),
            scratch_shapes=[
                pltpu.VMEM((1, D), BF16), pltpu.VMEM((1, D), BF16), pltpu.VMEM((FF,), BF16),
                pltpu.VMEM((D, 6 * D), BF16), pltpu.VMEM((D, H * DH), BF16),
                pltpu.VMEM((2, R, D), BF16), pltpu.VMEM((D, FF), BF16), pltpu.VMEM((NG, 2 * GR, D), BF16),
                pltpu.VMEM((2, 2, R, W), BF16),
                pltpu.VMEM((M, W), F32), pltpu.VMEM((M, D), F32), pltpu.VMEM((NG, M, 2 * GR), F32),
                pltpu.SemaphoreType.DMA((S_W2 + NG,)),
            ],
            compiler_params=pltpu.CompilerParams(vmem_limit_bytes=64 * 1024 * 1024, disable_semaphore_checks=nosem),
        )(A_x, kt, vt, A_wq, A_wo, B_w1, B_b1, B_w2, c, w_mod)
    return fn


@jax.jit
def pallas_adaLN_cond__sliding_block_cached__dense_activation_mish__decode_kernel(A_x, A_k_cache, A_v_cache, A_wq, A_wo, B_x, B_w1, B_b1, B_w2, c, w_mod):
    return make()(A_x, A_k_cache, A_v_cache, A_wq, A_wo, B_x, B_w1, B_b1, B_w2, c, w_mod)
```

```python
import jax
import jax.numpy as jnp
from jax import lax
import jax.experimental.pallas as pl
import jax.experimental.pallas.tpu as pltpu

F32 = jnp.float32
BF16 = jnp.bfloat16
N_HEADS, HEAD_DIM = 32, 192
M = 8
TR = 8


def _layernorm(x, eps=1e-5):
    m = jnp.mean(x, axis=-1, keepdims=True)
    d = x - m
    v = jnp.mean(d * d, axis=-1, keepdims=True)
    return d / jnp.sqrt(v + eps)


def _dot(a, b):
    return jnp.dot(a, b, preferred_element_type=F32)


def _dot_nt(a, b):
    return lax.dot_general(a, b, (((1,), (1,)), ((), ())), preferred_element_type=F32)


def _block_kernel(
    x_hbm, kt_hbm, vt_hbm, wq_hbm, wo_hbm, w1_hbm, b1_hbm, w2_hbm, c_hbm, wmod_hbm,
    o_ref,
    x_v, c_v, b1_v, wmod_v, wq_v, wo_v, w1_v, w2_v, kv_v, p_v, acc_v, act_v, sem,
):
    D, FF = w1_hbm.shape
    SK = kt_hbm.shape[1]
    R, W = kv_v.shape[2:]
    NP = kt_hbm.shape[0] // R
    KR, KC = 32, 512
    WO_ROWS, WO_WAYS = 24, 8
    W2_CUTS = (0, 7 * FF // 12, 5 * FF // 6, FF)

    kv_sem = lambda slot: sem.at[slot]
    wo_sem = lambda slot: sem.at[2 + slot]
    small_sem, wmod_sem, wq_sem = wo_sem(0), wo_sem(1), kv_sem(1)
    w1_sem = kv_sem(NP % 2)
    w2_sems = (kv_sem((NP + 1) % 2), wo_sem(0), wo_sem(1))

    def start(src, dst, s, queue):
        pltpu.make_async_copy(src, dst, s).start(priority=queue)

    def wait_filled(buf, s):
        pltpu.make_async_copy(buf, buf, s).wait()

    def fetch_weight(src, dst, s, rows, cols, ways, lo=0, hi=None):
        hi = src.shape[0] if hi is None else hi
        n = (hi - lo) // ways
        assert n * ways == hi - lo and n % rows == 0 and src.shape[1] % cols == 0
        for r in range(lo, lo + n, rows):
            for col in range(0, src.shape[1], cols):
                for way in range(ways):
                    idx = (pl.ds(r + way * n, rows), pl.ds(col, cols))
                    start(src.at[idx], dst.at[idx], s, way % 2)

    def fetch_heads(p, half):
        slot = p % 2
        rows = lambda r, n: pl.ds(pl.multiple_of(p * R + r, TR), n)
        blocks, steps = W // KC, R // KR
        for j in range(half * blocks // 2, (half + 1) * blocks // 2):
            kv, col = j % 2, j // 2 * 2 * KC
            for t in range(steps):
                for queue in range(2):
                    start((kt_hbm, vt_hbm)[kv].at[rows(t * KR, KR), pl.ds(SK - W + col + queue * KC, KC)],
                          kv_v.at[slot, kv, pl.ds(t * KR, KR), pl.ds(col + queue * KC, KC)],
                          kv_sem(slot), queue)

    def fetch_w2(g):
        fetch_weight(w2_hbm, w2_v, w2_sems[g], 32, D, 4 if g == 0 else 2,
                     W2_CUTS[g], W2_CUTS[g + 1])

    def ffn_out_part(g):
        rows = pl.ds(W2_CUTS[g], W2_CUTS[g + 1] - W2_CUTS[g])
        wait_filled(w2_v.at[rows], w2_sems[g])
        return _dot(act_v[:, rows].astype(BF16), w2_v[rows, :])

    small = [pltpu.make_async_copy(c_hbm, c_v, small_sem),
             pltpu.make_async_copy(x_hbm.at[0], x_v, small_sem),
             pltpu.make_async_copy(b1_hbm, b1_v, small_sem)]
    for i, copy in enumerate(small):
        copy.start(priority=(i + 1) % 2)
    fetch_weight(wmod_hbm, wmod_v, wmod_sem, TR, 2 * D, 8)
    fetch_weight(wq_hbm, wq_v, wq_sem, TR, 2048, 10)
    fetch_weight(wo_hbm, wo_v, sem.at[4], WO_ROWS, D, WO_WAYS)

    for copy in small:
        copy.wait()
    wait_filled(wmod_v, wmod_sem)
    c = jnp.broadcast_to(c_v[...].astype(F32), (M, D))
    mod = _dot((c * jax.nn.sigmoid(c)).astype(BF16), wmod_v[...])
    sa, ca, ga, sb, cb, gb = (mod[:, i * D:(i + 1) * D] for i in range(6))
    x = jnp.broadcast_to(x_v[...].astype(F32), (M, D))
    h = (_layernorm(x) * (1.0 + ca) + sa).astype(BF16)

    row = lax.broadcasted_iota(jnp.int32, (M, R), 0)
    col = lax.broadcasted_iota(jnp.int32, (M, R), 1)
    own_head = (col >= row * HEAD_DIM) & (col < (row + 1) * HEAD_DIM)
    acc_v[...] = jnp.zeros_like(acc_v)

    def step(i, carry):
        p = jnp.maximum(i - 1, 0)
        slot = p % 2

        @pl.when(i < NP)
        def _():
            fetch_heads(i, 0)

        @pl.when(i == NP)
        def _():
            fetch_weight(w1_hbm, w1_v, w1_sem, TR, FF, 4)

        @pl.when(i == 0)
        def _():
            wait_filled(wq_v, wq_sem)
            wait_filled(wo_v, sem.at[4])

        @pl.when(i > 0)
        def _():
            wait_filled(kv_v.at[slot], kv_sem(slot))
            q = _dot(h, wq_v[:, pl.ds(pl.multiple_of(p * R, 128), R)])
            q = jnp.where(own_head, q, 0.0).astype(BF16)
            s = _dot(q, kv_v[slot, 0]) * (HEAD_DIM ** -0.5)
            e = jnp.exp(s - jnp.max(s, axis=-1, keepdims=True))
            p_v[...] = e / jnp.sum(e, axis=-1, keepdims=True)

        @pl.when(i < NP)
        def _():
            fetch_heads(i, 1)

        @pl.when(i == NP)
        def _():
            fetch_w2(0)

        @pl.when(i > 0)
        def _():
            o = _dot_nt(p_v[...].astype(BF16), kv_v[slot, 1])
            o = jnp.where(own_head, o, 0.0).astype(BF16)
            acc_v[...] += _dot(o, wo_v[pl.ds(pl.multiple_of(p * R, R), R), :])

        return carry

    lax.fori_loop(0, NP + 1, step, 0)
    fetch_w2(1)
    fetch_w2(2)

    x = x + ga * jnp.sum(acc_v[...], axis=0, keepdims=True)
    h = (_layernorm(x) * (1.0 + cb) + sb).astype(BF16)
    wait_filled(w1_v, w1_sem)
    u = _dot(h, w1_v[...]) + b1_v[...].astype(F32).reshape(1, FF)
    softplus = jnp.log1p(jnp.exp(-jnp.abs(u))) + jnp.where(u > 0, u, 0.0)
    act_v[...] = u * jnp.tanh(softplus)
    acc_v[...] = jnp.zeros_like(acc_v)

    def early_parts(i, carry):
        for g in range(2):
            @pl.when(i == g)
            def _():
                acc_v[...] += ffn_out_part(g)
        return carry

    lax.fori_loop(0, 2, early_parts, 0)
    y = acc_v[...] + ffn_out_part(2)
    o_ref[0] = (x + gb * y)[0:1, :].astype(o_ref.dtype)


@jax.jit
def pallas_adaLN_cond__sliding_block_cached__dense_activation_mish__decode_kernel(
    A_x: jax.Array,
    A_k_cache: jax.Array,
    A_v_cache: jax.Array,
    A_wq: jax.Array,
    A_wo: jax.Array,
    B_x: jax.Array,
    B_w1: jax.Array,
    B_b1: jax.Array,
    B_w2: jax.Array,
    c: jax.Array,
    w_mod: jax.Array,
):
    del B_x
    D, FF = B_w1.shape
    SK = A_k_cache.shape[2]
    assert A_x.shape == (1, 1, D) and A_k_cache.shape == (1, N_HEADS, SK, HEAD_DIM)
    W = min(4096, max(256, SK // 4))
    R = 2 * HEAD_DIM

    kt = jnp.swapaxes(A_k_cache, 2, 3).reshape(N_HEADS * HEAD_DIM, SK)
    vt = jnp.swapaxes(A_v_cache, 2, 3).reshape(N_HEADS * HEAD_DIM, SK)
    return pl.pallas_call(
        _block_kernel,
        out_shape=jax.ShapeDtypeStruct(A_x.shape, A_x.dtype),
        in_specs=[pl.BlockSpec(memory_space=pltpu.HBM)] * 10,
        out_specs=pl.BlockSpec(memory_space=pltpu.VMEM),
        scratch_shapes=[
            pltpu.VMEM((1, D), A_x.dtype),
            pltpu.VMEM((1, D), c.dtype),
            pltpu.VMEM(B_b1.shape, B_b1.dtype),
            pltpu.VMEM(w_mod.shape, w_mod.dtype),
            pltpu.VMEM(A_wq.shape, A_wq.dtype),
            pltpu.VMEM(A_wo.shape, A_wo.dtype),
            pltpu.VMEM(B_w1.shape, B_w1.dtype),
            pltpu.VMEM(B_w2.shape, B_w2.dtype),
            pltpu.VMEM((2, 2, R, W), A_k_cache.dtype),
            pltpu.VMEM((M, W), F32),
            pltpu.VMEM((M, D), F32),
            pltpu.VMEM((M, FF), F32),
            pltpu.SemaphoreType.DMA((5,)),
        ],
        compiler_params=pltpu.CompilerParams(vmem_limit_bytes=64 * 1024 * 1024),
    )(A_x, kt, vt, A_wq, A_wo, B_w1, B_b1, B_w2, c, w_mod)
```

```python
import jax
import jax.numpy as jnp
from jax import lax
import jax.experimental.pallas as pl
import jax.experimental.pallas.tpu as pltpu

F32 = jnp.float32
BF16 = jnp.bfloat16
N_HEADS, HEAD_DIM = 32, 192
M = 8
TR = 8


def _layernorm(x, eps=1e-5):
    m = jnp.mean(x, axis=-1, keepdims=True)
    d = x - m
    v = jnp.mean(d * d, axis=-1, keepdims=True)
    return d / jnp.sqrt(v + eps)


def _dot(a, b):
    return jnp.dot(a, b, preferred_element_type=F32)


def _dot_nt(a, b):
    return lax.dot_general(a, b, (((1,), (1,)), ((), ())), preferred_element_type=F32)


def _block_kernel(
    x_hbm, kt_hbm, vt_hbm, wq_hbm, wo_hbm, w1_hbm, b1_hbm, w2_hbm, c_hbm, wmod_hbm,
    o_ref,
    x_v, c_v, b1_v, wmod_v, wq_v, wo_v, w1_v, w2_v, kv_v, p_v, acc_v, act_v, sem,
):
    D, FF = w1_hbm.shape
    SK = kt_hbm.shape[1]
    R, W = kv_v.shape[2:]
    NP = kt_hbm.shape[0] // R
    KR, KC = 32, 512
    W2_CUTS = (0, 7 * FF // 12, 5 * FF // 6, FF)

    kv_sem = lambda slot: sem.at[slot]
    wq_sem, w1_sem = kv_sem(1), kv_sem(NP % 2)
    small_sem, wmod_sem, wo_sem = w2_sems = (sem.at[2], sem.at[3], sem.at[4])

    def start(src, dst, s, queue):
        pltpu.make_async_copy(src, dst, s).start(priority=queue)

    def wait_filled(buf, s):
        pltpu.make_async_copy(buf, buf, s).wait()

    def fetch_weight(src, dst, s, rows, cols, ways, lo=0, hi=None):
        hi = src.shape[0] if hi is None else hi
        n = (hi - lo) // ways
        assert n * ways == hi - lo and n % rows == 0 and src.shape[1] % cols == 0
        for r in range(lo, lo + n, rows):
            for col in range(0, src.shape[1], cols):
                for way in range(ways):
                    idx = (pl.ds(r + way * n, rows), pl.ds(col, cols))
                    start(src.at[idx], dst.at[idx], s, way % 2)

    def fetch_heads(p, half):
        slot = p % 2
        assert W % (4 * KC) == 0 and R % KR == 0
        for col in range(half * W // 2, (half + 1) * W // 2, 2 * KC):
            for kv, src in enumerate((kt_hbm, vt_hbm)):
                for r in range(0, R, KR):
                    rows = pl.ds(pl.multiple_of(p * R + r, TR), KR)
                    for queue in range(2):
                        at = col + queue * KC
                        start(src.at[rows, pl.ds(SK - W + at, KC)],
                              kv_v.at[slot, kv, pl.ds(r, KR), pl.ds(at, KC)],
                              kv_sem(slot), queue)

    def fetch_w2(g):
        fetch_weight(w2_hbm, w2_v, w2_sems[g], 4 * TR, D, 4 if g == 0 else 2,
                     W2_CUTS[g], W2_CUTS[g + 1])

    def ffn_out_part(g):
        rows = pl.ds(W2_CUTS[g], W2_CUTS[g + 1] - W2_CUTS[g])
        wait_filled(w2_v.at[rows], w2_sems[g])
        return _dot(act_v[:, rows].astype(BF16), w2_v[rows, :])

    small = [pltpu.make_async_copy(c_hbm, c_v, small_sem),
             pltpu.make_async_copy(x_hbm.at[0], x_v, small_sem),
             pltpu.make_async_copy(b1_hbm, b1_v, small_sem)]
    for i, copy in enumerate(small):
        copy.start(priority=(i + 1) % 2)
    fetch_weight(wmod_hbm, wmod_v, wmod_sem, TR, 2 * D, 8)
    fetch_weight(wq_hbm, wq_v, wq_sem, TR, 2048, 10)
    fetch_weight(wo_hbm, wo_v, wo_sem, 3 * TR, D, 8)

    for copy in small:
        copy.wait()
    wait_filled(wmod_v, wmod_sem)
    c = jnp.broadcast_to(c_v[...].astype(F32), (M, D))
    mod = _dot((c * jax.nn.sigmoid(c)).astype(BF16), wmod_v[...])
    sa, ca, ga, sb, cb, gb = (mod[:, i * D:(i + 1) * D] for i in range(6))
    x = jnp.broadcast_to(x_v[...].astype(F32), (M, D))
    h = (_layernorm(x) * (1.0 + ca) + sa).astype(BF16)

    row = lax.broadcasted_iota(jnp.int32, (M, R), 0)
    col = lax.broadcasted_iota(jnp.int32, (M, R), 1)
    own_head = (col >= row * HEAD_DIM) & (col < (row + 1) * HEAD_DIM)
    acc_v[...] = jnp.zeros_like(acc_v)

    def step(i, carry):
        p = jnp.maximum(i - 1, 0)
        slot = p % 2

        @pl.when(i < NP)
        def _():
            fetch_heads(i, 0)

        @pl.when(i == NP)
        def _():
            fetch_weight(w1_hbm, w1_v, w1_sem, TR, FF, 4)

        @pl.when(i == 0)
        def _():
            wait_filled(wq_v, wq_sem)
            wait_filled(wo_v, wo_sem)

        @pl.when(i > 0)
        def _():
            wait_filled(kv_v.at[slot], kv_sem(slot))
            q = _dot(h, wq_v[:, pl.ds(pl.multiple_of(p * R, 128), R)])
            q = jnp.where(own_head, q, 0.0).astype(BF16)
            s = _dot(q, kv_v[slot, 0]) * (HEAD_DIM ** -0.5)
            e = jnp.exp(s - jnp.max(s, axis=-1, keepdims=True))
            p_v[...] = e / jnp.sum(e, axis=-1, keepdims=True)

        @pl.when(i < NP)
        def _():
            fetch_heads(i, 1)

        @pl.when(i == NP)
        def _():
            fetch_w2(0)

        @pl.when(i > 0)
        def _():
            o = _dot_nt(p_v[...].astype(BF16), kv_v[slot, 1])
            o = jnp.where(own_head, o, 0.0).astype(BF16)
            acc_v[...] += _dot(o, wo_v[pl.ds(pl.multiple_of(p * R, R), R), :])

        return carry

    lax.fori_loop(0, NP + 1, step, 0)
    fetch_w2(1)
    fetch_w2(2)

    x = x + ga * jnp.sum(acc_v[...], axis=0, keepdims=True)
    h = (_layernorm(x) * (1.0 + cb) + sb).astype(BF16)
    wait_filled(w1_v, w1_sem)
    u = _dot(h, w1_v[...]) + b1_v[...].astype(F32).reshape(1, FF)
    softplus = jnp.log1p(jnp.exp(-jnp.abs(u))) + jnp.where(u > 0, u, 0.0)
    act_v[...] = u * jnp.tanh(softplus)
    acc_v[...] = jnp.zeros_like(acc_v)

    def early_parts(i, carry):
        for g in range(2):
            @pl.when(i == g)
            def _():
                acc_v[...] += ffn_out_part(g)
        return carry

    lax.fori_loop(0, 2, early_parts, 0)
    y = acc_v[...] + ffn_out_part(2)
    o_ref[0] = (x + gb * y)[0:1, :].astype(o_ref.dtype)


@jax.jit
def pallas_adaLN_cond__sliding_block_cached__dense_activation_mish__decode_kernel(
    A_x: jax.Array,
    A_k_cache: jax.Array,
    A_v_cache: jax.Array,
    A_wq: jax.Array,
    A_wo: jax.Array,
    B_x: jax.Array,
    B_w1: jax.Array,
    B_b1: jax.Array,
    B_w2: jax.Array,
    c: jax.Array,
    w_mod: jax.Array,
):
    del B_x
    D, FF = B_w1.shape
    SK = A_k_cache.shape[2]
    assert A_x.shape == (1, 1, D) and A_k_cache.shape == (1, N_HEADS, SK, HEAD_DIM)
    W = min(4096, max(256, SK // 4))
    R = 2 * HEAD_DIM

    kt = jnp.swapaxes(A_k_cache, 2, 3).reshape(N_HEADS * HEAD_DIM, SK)
    vt = jnp.swapaxes(A_v_cache, 2, 3).reshape(N_HEADS * HEAD_DIM, SK)
    return pl.pallas_call(
        _block_kernel,
        out_shape=jax.ShapeDtypeStruct(A_x.shape, A_x.dtype),
        in_specs=[pl.BlockSpec(memory_space=pltpu.HBM)] * 10,
        out_specs=pl.BlockSpec(memory_space=pltpu.VMEM),
        scratch_shapes=[
            pltpu.VMEM((1, D), A_x.dtype),
            pltpu.VMEM((1, D), c.dtype),
            pltpu.VMEM(B_b1.shape, B_b1.dtype),
            pltpu.VMEM(w_mod.shape, w_mod.dtype),
            pltpu.VMEM(A_wq.shape, A_wq.dtype),
            pltpu.VMEM(A_wo.shape, A_wo.dtype),
            pltpu.VMEM(B_w1.shape, B_w1.dtype),
            pltpu.VMEM(B_w2.shape, B_w2.dtype),
            pltpu.VMEM((2, 2, R, W), A_k_cache.dtype),
            pltpu.VMEM((M, W), F32),
            pltpu.VMEM((M, D), F32),
            pltpu.VMEM((M, FF), F32),
            pltpu.SemaphoreType.DMA((5,)),
        ],
        compiler_params=pltpu.CompilerParams(vmem_limit_bytes=64 * 1024 * 1024),
    )(A_x, kt, vt, A_wq, A_wo, B_w1, B_b1, B_w2, c, w_mod)
```
